```python
import os as _os
_os.environ.setdefault("JAX_PLATFORMS", "cpu")
import jax
import jax.numpy as jnp

def _softmax(x, axis=-1):
    return jax.nn.softmax(x, axis=axis)
def _gelu(x):
    return jax.nn.gelu(x, approximate=True)
def _silu(x):
    return jax.nn.silu(x)
def _sigmoid(x):
    return jax.nn.sigmoid(x)
def _layernorm(x, axis=-1, eps=1e-5):
    m = jnp.mean(x, axis=axis, keepdims=True)
    v = jnp.var(x, axis=axis, keepdims=True)
    return (x - m) / jnp.sqrt(v + eps)
def _scatter_add(tgt, idx, src, axis=0):
    return tgt.at[idx].add(src)
def _segment_sum(src, seg, n):
    return jax.ops.segment_sum(src, seg, n)
class _Rng:
    def __init__(self, key):
        self._k = key
    def _next(self):
        self._k, sub = jax.random.split(self._k)
        return sub
    def normal(self, shape):
        return jax.random.normal(self._next(), shape, dtype=jnp.bfloat16)
    def randint(self, lo, hi, shape):
        return jax.random.randint(self._next(), shape, lo, hi, dtype=jnp.int32)
    def uniform(self, shape, lo=0.0, hi=1.0):
        return jax.random.uniform(self._next(), shape, jnp.bfloat16, lo, hi)
    def permutation(self, n):
        return jax.random.permutation(self._next(), n)


kernel_name = 'standalone__mha_softmax__near_ridge'

def setup_inputs():
    _rng = _Rng(jax.random.key(int.from_bytes(__import__("os").urandom(4), "little")))
    _w = (lambda a: (lambda t: t.astype(jnp.bfloat16) if jnp.issubdtype(t.dtype, jnp.floating) else t)(jnp.asarray(a)))
    B, H, Sq, Sk, D = 8, 32, 384, 512, 128
    return {
        "q": _w((lambda *s: _rng.normal(s) * 0.4)(B, H, Sq, D)),
        "k": _w((lambda *s: _rng.normal(s) * 0.4)(B, H, Sk, D)),
        "v": _w((lambda *s: _rng.normal(s) * 0.05)(B, H, Sk, D)),
    }

def reference(q, k, v):
    scale = q.shape[-1] ** -0.5
    scores = jnp.einsum("bhqd,bhkd->bhqk", q, k) * scale
    p = _softmax(scores, axis=-1)
    return jnp.einsum("bhqk,bhkd->bhqd", p, v)
```

```python
import jax
import jax.numpy as jnp
from jax import lax
import jax.experimental.pallas as pl
import jax.experimental.pallas.tpu as pltpu

_LOG2E = 1.4426950408889634
_HEADS_PER_STEP = 8
_READ_ROWS = 16
_READS_PER_STEP = 39
_READ_STEPS = 25
_WRITE_HEADS = 32
_WRITE_ROWS = 16
_WRITES_PER_STEP = 24


def _attention_kernel(q_hbm, k_hbm, v_hbm, o_hbm, qb, kb, vb, ob, rsem, wsem):
  n_heads, s_k, d = kb.shape
  s_q = ob.shape[1]
  hs, rr, wr, wh = _HEADS_PER_STEP, _READ_ROWS, _WRITE_ROWS, _WRITE_HEADS
  n_steps = n_heads // hs
  per_read = s_k // rr
  per_write = s_q // wr
  q_slabs = hs * s_q // s_k
  n_pre = n_steps * per_read - _READS_PER_STEP * _READ_STEPS
  n_in_loop = _WRITES_PER_STEP * (n_steps - _READ_STEPS)
  n_writes = n_heads // wh * per_write
  scale = d**-0.5 * _LOG2E

  def spread(n):
    return [[j for j in range(n) if j * hs // n == u] for u in range(hs)]

  for x in range(n_in_loop):
    step, j = divmod(x, _WRITES_PER_STEP)
    done = (_READ_STEPS + step) * hs + j * hs // _WRITES_PER_STEP
    assert (x // per_write + 1) * wh <= done
  for i in range(min(_READ_STEPS + 1, n_steps)):
    assert n_pre + _READS_PER_STEP * i >= per_read * (i + 1)
  assert n_in_loop % 2 == 0 and n_writes % 2 == 0

  inputs = ((k_hbm, kb, hs), (q_hbm, qb, q_slabs), (v_hbm, vb, hs))

  def start_read(x, j):
    g = lax.div(x, per_read)
    rows = pl.ds(pl.multiple_of(lax.rem(x, per_read) * rr, rr), rr)
    for a, (hbm, buf, n) in enumerate(inputs):
      slabs = pl.ds(g * n, n)
      pltpu.make_async_copy(
          hbm.at[slabs, rows], buf.at[slabs, rows], rsem.at[a, g]
      ).start(priority=(j + a) % 2)

  def wait_read(g):
    for a, (_, buf, n) in enumerate(inputs):
      group = buf.at[pl.ds(g * n, n)]
      pltpu.make_async_copy(group, group, rsem.at[a, g]).wait()

  def start_write(x, j):
    heads = pl.ds(lax.div(x, per_write) * wh, wh)
    rows = pl.ds(pl.multiple_of(lax.rem(x, per_write) * wr, wr), wr)
    pltpu.make_async_copy(
        ob.at[heads, rows], o_hbm.at[heads, rows], wsem.at[0]
    ).start(priority=j % 2)

  def attend(h):
    pieces = []
    for t in range(s_q // 128):
      row = h * s_q + t * 128
      rows = pl.ds(pl.multiple_of(lax.rem(row, s_k), 128), 128)
      pieces.append(qb[lax.div(row, s_k), rows])
    q = jnp.concatenate(pieces, axis=0)
    s = lax.dot_general(
        q, kb[h], (((1,), (1,)), ((), ())),
        preferred_element_type=jnp.float32,
    )
    m = jnp.max(s, axis=-1, keepdims=True)
    p = jnp.exp2((s - m) * scale)
    l = jnp.sum(p, axis=-1, keepdims=True)
    v = vb[h]
    o = jnp.dot(p.astype(v.dtype), v, preferred_element_type=jnp.float32)
    ob[h] = (o * pltpu.reciprocal(l, approx=True)).astype(ob.dtype)

  @pl.loop(0, n_pre // 2)
  def _(x):
    start_read(2 * x, 0)
    start_read(2 * x + 1, 1)

  if n_pre % 2:
    start_read(n_pre - 1, 0)

  @pl.loop(0, _READ_STEPS)
  def _(i):
    wait_read(i)
    for u, js in enumerate(spread(_READS_PER_STEP)):
      attend(i * hs + u)
      for j in js:
        start_read(n_pre + i * _READS_PER_STEP + j, j)

  @pl.loop(_READ_STEPS, n_steps)
  def _(i):
    wait_read(i)
    for u, js in enumerate(spread(_WRITES_PER_STEP)):
      for j in js:
        start_write((i - _READ_STEPS) * _WRITES_PER_STEP + j, j)
      attend(i * hs + u)

  @pl.loop(n_in_loop // 2, n_writes // 2)
  def _(x):
    start_write(2 * x, 0)
    start_write(2 * x + 1, 1)

  pltpu.make_async_copy(ob, ob, wsem.at[0]).wait()


@jax.jit
def pallas_standalone__mha_softmax__near_ridge_kernel(
    q: jax.Array,
    k: jax.Array,
    v: jax.Array,
):
  b, h, s_q, d = q.shape
  s_k = k.shape[2]
  n = b * h
  q_shape = (n * s_q // s_k, s_k, d)
  out = pl.pallas_call(
      _attention_kernel,
      in_specs=[pl.BlockSpec(memory_space=pl.ANY)] * 3,
      out_specs=pl.BlockSpec(memory_space=pl.ANY),
      out_shape=jax.ShapeDtypeStruct((n, s_q, d), q.dtype),
      scratch_shapes=[
          pltpu.VMEM(q_shape, q.dtype),
          pltpu.VMEM((n, s_k, d), k.dtype),
          pltpu.VMEM((n, s_k, d), v.dtype),
          pltpu.VMEM((n, s_q, d), q.dtype),
          pltpu.SemaphoreType.DMA((3, n // _HEADS_PER_STEP)),
          pltpu.SemaphoreType.DMA((1,)),
      ],
      compiler_params=pltpu.CompilerParams(
          vmem_limit_bytes=124 << 20, disable_bounds_checks=True
      ),
  )(q.reshape(q_shape), k.reshape(n, s_k, d), v.reshape(n, s_k, d))
  return out.reshape(b, h, s_q, d)
```

```python
import functools

import jax
from jax import lax
import jax.experimental.pallas as pl
import jax.experimental.pallas.tpu as pltpu
import jax.numpy as jnp

_LOG2E = 1.4426950408889634
_SLABS = 8
_ROWS = 128
_READS_BEFORE = (64, 48, 64)
_READS_PER_STEP = (40, 30, 40)
_WRITES_PER_STEP = 102


def _read_order(counts):
  blocks = sorted(
      ((j // _SLABS + a / len(counts)) * _SLABS / n, a, j)
      for a, n in enumerate(counts)
      for j in range(n)
  )
  return [(pos, a, j) for pos, (_, a, j) in enumerate(blocks)]


def _attention_kernel(q_hbm, k_hbm, v_hbm, o_hbm, qb, kb, vb, ob, rsem, wsem):
  n_steps_x_sk, d = kb.shape[1:]
  inputs = ((k_hbm, kb), (q_hbm, qb), (v_hbm, vb))
  n_steps = rsem.shape[1]
  s_k = n_steps_x_sk // n_steps
  s_q = qb.shape[1] // n_steps
  scale = d**-0.5 * _LOG2E

  step_rows = (s_k, s_q, s_k)
  step_copies = tuple(r // _ROWS * _SLABS for r in step_rows)
  total_copies = tuple(n_steps * n for n in step_copies)
  out_copies = step_copies[1]

  order = _read_order(_READS_PER_STEP)
  reads = [[] for _ in range(_SLABS)]
  for pos, a, j in order:
    reads[(2 * pos + 1) * _SLABS // (2 * len(order))].append((a, j, pos % 2))
  writes = [[] for _ in range(_SLABS)]
  for j in range(_WRITES_PER_STEP):
    writes[j // 2 * 2 * _SLABS // _WRITES_PER_STEP].append(j)

  def read_index(i, a, j):
    return _READS_BEFORE[a] + i * _READS_PER_STEP[a] + j

  last_i, last_u = max(
      (i, u)
      for i in range(n_steps)
      for u in range(_SLABS)
      for a, j, _ in reads[u]
      if read_index(i, a, j) < total_copies[a]
  )
  write_lag = last_i * _WRITES_PER_STEP + (
      writes[last_u + 1][0] if last_u + 1 < _SLABS else _WRITES_PER_STEP
  )

  def first_write(i, minimum):
    return minimum(i * _WRITES_PER_STEP - write_lag, (i - 1) * out_copies)

  for a in range(len(inputs)):
    started = list(range(_READS_BEFORE[a]))
    for i in range(n_steps):
      assert len(started) >= (i + 1) * step_copies[a]
      started += [
          read_index(i, b, j)
          for slot in reads
          for b, j, _ in slot
          if b == a and read_index(i, b, j) < total_copies[a]
      ]
    assert sorted(started) == list(range(total_copies[a]))
  started = [
      first_write(i, min) + j
      for i in range(n_steps)
      for j in range(_WRITES_PER_STEP)
      if 0 <= first_write(i, min) + j < i * out_copies
  ]
  writes_in_loop = len(started)
  assert started == list(range(writes_in_loop)) and writes_in_loop % 2 == 0

  def block(x):
    start = pl.multiple_of(lax.div(x, _SLABS) * _ROWS, _ROWS)
    return lax.rem(x, _SLABS), pl.ds(start, _ROWS)

  def start_read(a, x, priority):
    hbm, buf = inputs[a]
    at = block(x)
    sem = rsem.at[a, lax.div(x, step_copies[a])]
    pltpu.make_async_copy(hbm.at[at], buf.at[at], sem).start(priority=priority)

  def wait_reads(i):
    for a, (_, buf) in enumerate(inputs):
      n = step_rows[a]
      rows = buf.at[:, pl.ds(pl.multiple_of(i * n, n), n)]
      pltpu.make_async_copy(rows, rows, rsem.at[a, i]).wait()

  def start_write(x, priority):
    at = block(x)
    pltpu.make_async_copy(ob.at[at], o_hbm.at[at], wsem.at[0]).start(
        priority=priority
    )

  def attend(u, i):
    q_rows = pl.ds(pl.multiple_of(i * s_q, _ROWS), s_q)
    k_rows = pl.ds(pl.multiple_of(i * s_k, _ROWS), s_k)
    s = lax.dot_general(
        qb[u, q_rows],
        kb[u, k_rows],
        (((1,), (1,)), ((), ())),
        preferred_element_type=jnp.float32,
    )
    m = jnp.max(s, axis=-1, keepdims=True)
    p = jnp.exp2((s - m) * scale)
    l = jnp.sum(p, axis=-1, keepdims=True)
    o = jnp.dot(
        p.astype(vb.dtype), vb[u, k_rows], preferred_element_type=jnp.float32
    )
    inv = pltpu.reciprocal(l, approx=False, full_range=False)
    ob[u, q_rows] = (o * inv).astype(ob.dtype)

  n_rounds = _READS_BEFORE[0] // _SLABS // 2
  per_round = tuple(n // n_rounds for n in _READS_BEFORE)
  assert tuple(n * n_rounds for n in per_round) == _READS_BEFORE

  @pl.loop(0, n_rounds)
  def _(t):
    for pos, a, j in _read_order(per_round):
      start_read(a, t * per_round[a] + j, pos % 2)

  @pl.loop(0, n_steps)
  def _(i):
    wait_reads(i)
    for u in range(_SLABS):
      for j in writes[u]:
        x = first_write(i, jnp.minimum) + j
        pl.when(x.astype(jnp.uint32) < i * out_copies)(
            functools.partial(start_write, x, j % 2)
        )
      attend(u, i)
      for a, j, priority in reads[u]:
        x = read_index(i, a, j)
        pl.when(x < total_copies[a])(
            functools.partial(start_read, a, x, priority)
        )

  @pl.loop(writes_in_loop // 2, n_steps * out_copies // 2)
  def _(t):
    start_write(2 * t, 0)
    start_write(2 * t + 1, 1)

  pltpu.make_async_copy(ob, ob, wsem.at[0]).wait()


@jax.jit
def pallas_standalone__mha_softmax__near_ridge_kernel(
    q: jax.Array,
    k: jax.Array,
    v: jax.Array,
):
  b, h, s_q, d = q.shape
  s_k = k.shape[2]
  n_steps = b * h // _SLABS
  q_shape = (_SLABS, n_steps * s_q, d)
  k_shape = (_SLABS, n_steps * s_k, d)
  out = pl.pallas_call(
      _attention_kernel,
      in_specs=[pl.BlockSpec(memory_space=pl.ANY)] * 3,
      out_specs=pl.BlockSpec(memory_space=pl.ANY),
      out_shape=jax.ShapeDtypeStruct(q_shape, q.dtype),
      scratch_shapes=[
          pltpu.VMEM(q_shape, q.dtype),
          pltpu.VMEM(k_shape, k.dtype),
          pltpu.VMEM(k_shape, v.dtype),
          pltpu.VMEM(q_shape, q.dtype),
          pltpu.SemaphoreType.DMA((3, n_steps)),
          pltpu.SemaphoreType.DMA((1,)),
      ],
      compiler_params=pltpu.CompilerParams(
          vmem_limit_bytes=124 << 20,
          disable_bounds_checks=True,
          disable_semaphore_checks=True,
      ),
  )(q.reshape(q_shape), k.reshape(k_shape), v.reshape(k_shape))
  return out.reshape(b, h, s_q, d)
```

```python
import functools

import jax
from jax import lax
import jax.experimental.pallas as pl
import jax.experimental.pallas.tpu as pltpu
import jax.numpy as jnp

_LOG2E = 1.4426950408889634
_SLABS = 8
_ROWS = 128
_WRITE_SLABS = 4
_READS_BEFORE = (64, 48, 64)
_READS_PER_STEP = (40, 30, 40)
_WRITES_PER_STEP = 102


def _divmod(x, n):
  assert n & (n - 1) == 0
  return lax.shift_right_logical(x, n.bit_length() - 1), x & (n - 1)


def _read_order(counts):
  blocks = sorted(
      ((j // _SLABS + a / len(counts)) * _SLABS / n, a, j)
      for a, n in enumerate(counts)
      for j in range(n)
  )
  return [(pos, a, j) for pos, (_, a, j) in enumerate(blocks)]


def _attention_kernel(q_hbm, k_hbm, v_hbm, o_hbm, qb, kb, vb, ob, rsem, wsem):
  inputs = ((k_hbm, kb), (q_hbm, qb), (v_hbm, vb))
  n_steps = rsem.shape[1]
  s_q = qb.shape[1] // n_steps
  s_k = kb.shape[1] // n_steps
  scale = qb.shape[2] ** -0.5 * _LOG2E

  step_rows = (s_k, s_q, s_k)
  step_copies = tuple(r // _ROWS * _SLABS for r in step_rows)
  total_copies = tuple(n_steps * n for n in step_copies)
  out_copies = step_copies[1]

  order = _read_order(_READS_PER_STEP)
  reads = [[] for _ in range(_SLABS)]
  for pos, a, j in order:
    reads[(2 * pos + 1) * _SLABS // (2 * len(order))].append((a, j, pos % 2))
  writes = [[] for _ in range(_SLABS)]
  for j in range(_WRITES_PER_STEP):
    writes[j // 2 * 2 * _SLABS // _WRITES_PER_STEP].append(j)

  def read_index(i, a, j):
    return _READS_BEFORE[a] + i * _READS_PER_STEP[a] + j

  last_i, last_u = max(
      (i, u)
      for i in range(n_steps)
      for u in range(_SLABS)
      for a, j, _ in reads[u]
      if read_index(i, a, j) < total_copies[a]
  )
  write_lag = last_i * _WRITES_PER_STEP + (
      writes[last_u + 1][0] if last_u + 1 < _SLABS else _WRITES_PER_STEP
  )

  def first_write(i, minimum):
    return minimum(i * _WRITES_PER_STEP - write_lag, (i - 1) * out_copies)

  for a in range(len(inputs)):
    started = list(range(_READS_BEFORE[a]))
    for i in range(n_steps):
      assert len(started) >= (i + 1) * step_copies[a]
      started += [
          read_index(i, b, j)
          for slot in reads
          for b, j, _ in slot
          if b == a and read_index(i, b, j) < total_copies[a]
      ]
    assert sorted(started) == list(range(total_copies[a]))
  started = [
      first_write(i, min) + j
      for i in range(n_steps)
      for j in range(_WRITES_PER_STEP)
      if 0 <= first_write(i, min) + j < i * out_copies
  ]
  writes_in_loop = len(started)
  assert started == list(range(writes_in_loop)) and writes_in_loop % 2 == 0

  def start_read(a, x, priority):
    hbm, buf = inputs[a]
    block, slab = _divmod(x, _SLABS)
    at = (slab, pl.ds(pl.multiple_of(block * _ROWS, _ROWS), _ROWS))
    sem = rsem.at[a, lax.div(x, step_copies[a])]
    pltpu.make_async_copy(hbm.at[at], buf.at[at], sem).start(priority=priority)

  def wait_reads(i):
    for a, (hbm, buf) in enumerate(inputs):
      rows = pl.ds(pl.multiple_of(i * step_rows[a], _ROWS), step_rows[a])
      pltpu.make_async_copy(
          hbm.at[:, rows], buf.at[:, rows], rsem.at[a, i]
      ).wait()

  def start_write(x, priority):
    block, group = _divmod(x, _SLABS // _WRITE_SLABS)
    rows = _ROWS // _WRITE_SLABS
    at = (
        pl.ds(group * _WRITE_SLABS, _WRITE_SLABS),
        pl.ds(pl.multiple_of(block * rows, rows), rows),
    )
    pltpu.make_async_copy(ob.at[at], o_hbm.at[at], wsem.at[0]).start(
        priority=priority
    )

  def attend(u, i):
    q_rows = pl.ds(pl.multiple_of(i * s_q, _ROWS), s_q)
    k_rows = pl.ds(pl.multiple_of(i * s_k, _ROWS), s_k)
    s = lax.dot_general(
        qb[u, q_rows],
        kb[u, k_rows],
        (((1,), (1,)), ((), ())),
        preferred_element_type=jnp.float32,
    )
    m = jnp.max(s, axis=-1, keepdims=True)
    p = jnp.exp2((s - m) * scale)
    l = jnp.sum(p, axis=-1, keepdims=True)
    o = jnp.dot(
        p.astype(vb.dtype), vb[u, k_rows], preferred_element_type=jnp.float32
    )
    inv = pltpu.reciprocal(l, approx=False, full_range=False)
    ob[u, q_rows] = (o * inv).astype(ob.dtype)

  for pos, a, j in _read_order(_READS_BEFORE):
    start_read(a, jnp.int32(j), pos % 2)

  @pl.loop(0, n_steps)
  def _(i):
    wait_reads(i)
    for u in range(_SLABS):
      for j in writes[u]:
        x = first_write(i, jnp.minimum) + j
        pl.when((x >= 0) & (x < i * out_copies))(
            functools.partial(start_write, x, j % 2)
        )
      attend(u, i)
      for a, j, priority in reads[u]:
        x = read_index(i, a, j)
        pl.when(x < total_copies[a])(
            functools.partial(start_read, a, x, priority)
        )

  @pl.loop(writes_in_loop // 2, n_steps * out_copies // 2)
  def _(t):
    start_write(2 * t, 0)
    start_write(2 * t + 1, 1)

  pltpu.make_async_copy(ob, o_hbm, wsem.at[0]).wait()


@jax.jit
def pallas_standalone__mha_softmax__near_ridge_kernel(
    q: jax.Array,
    k: jax.Array,
    v: jax.Array,
):
  b, h, s_q, d = q.shape
  s_k = k.shape[2]
  n_steps = b * h // _SLABS
  q_shape = (_SLABS, n_steps * s_q, d)
  k_shape = (_SLABS, n_steps * s_k, d)
  out = pl.pallas_call(
      _attention_kernel,
      in_specs=[pl.BlockSpec(memory_space=pl.ANY)] * 3,
      out_specs=pl.BlockSpec(memory_space=pl.ANY),
      out_shape=jax.ShapeDtypeStruct(q_shape, q.dtype),
      scratch_shapes=[
          pltpu.VMEM(q_shape, q.dtype),
          pltpu.VMEM(k_shape, k.dtype),
          pltpu.VMEM(k_shape, v.dtype),
          pltpu.VMEM(q_shape, q.dtype),
          pltpu.SemaphoreType.DMA((3, n_steps)),
          pltpu.SemaphoreType.DMA((1,)),
      ],
      compiler_params=pltpu.CompilerParams(
          vmem_limit_bytes=124 << 20,
          disable_bounds_checks=True,
          disable_semaphore_checks=True,
      ),
  )(q.reshape(q_shape), k.reshape(k_shape), v.reshape(k_shape))
  return out.reshape(b, h, s_q, d)
```
